```python
import os as _os
_os.environ.setdefault("JAX_PLATFORMS", "cpu")
import jax
import jax.numpy as jnp

def _softmax(x, axis=-1):
    return jax.nn.softmax(x, axis=axis)
def _gelu(x):
    return jax.nn.gelu(x, approximate=True)
def _silu(x):
    return jax.nn.silu(x)
def _sigmoid(x):
    return jax.nn.sigmoid(x)
def _layernorm(x, axis=-1, eps=1e-5):
    m = jnp.mean(x, axis=axis, keepdims=True)
    v = jnp.var(x, axis=axis, keepdims=True)
    return (x - m) / jnp.sqrt(v + eps)
def _scatter_add(tgt, idx, src, axis=0):
    return tgt.at[idx].add(src)
def _segment_sum(src, seg, n):
    return jax.ops.segment_sum(src, seg, n)
class _Rng:
    def __init__(self, key):
        self._k = key
    def _next(self):
        self._k, sub = jax.random.split(self._k)
        return sub
    def normal(self, shape):
        return jax.random.normal(self._next(), shape, dtype=jnp.bfloat16)
    def randint(self, lo, hi, shape):
        return jax.random.randint(self._next(), shape, lo, hi, dtype=jnp.int32)
    def uniform(self, shape, lo=0.0, hi=1.0):
        return jax.random.uniform(self._next(), shape, jnp.bfloat16, lo, hi)
    def permutation(self, n):
        return jax.random.permutation(self._next(), n)


kernel_name = 'sequential_preLN__compressed_kv_cla__dense_activation_mish__decode'

def setup_inputs():
    _rng = _Rng(jax.random.key(int.from_bytes(__import__("os").urandom(4), "little")))
    _w = (lambda a: (lambda t: t.astype(jnp.bfloat16) if jnp.issubdtype(t.dtype, jnp.floating) else t)(jnp.asarray(a)))
    def _A_setup():
        B, H, Sq, Sk, D, M = 2, 32, 1, 8192, 128, 512
        Dc = 4 * D
        return {
            "x": _w((lambda *s: _rng.normal(s) * 0.05)(B, Sq, M)),
            "c_kv": _w((lambda *s: _rng.normal(s) * 0.8)(B, Sk, Dc)),
            "w_q": _w((lambda *s: _rng.normal(s) * 0.8)(M, H, D) * (M ** -0.5)),
            "w_uk": _w((lambda *s: _rng.normal(s) * 0.8)(Dc, H, D) * (Dc ** -0.5)),
            "w_uv": _w((lambda *s: _rng.normal(s) * 0.8)(Dc, H, D) * (Dc ** -0.5)),
            "w_o": _w((lambda *s: _rng.normal(s) * 0.8)(H, D, M) * ((H * D) ** -0.5)),
        }
    _A_in = _A_setup()

    def _B_setup():
        B, S, D, F = 2, 1, 512, 1792
        return {
            "x": _w((lambda *s: _rng.normal(s) * 0.05)(B, S, D)),
            "w1": _w((lambda *s: _rng.normal(s) * 0.4)(D, F) * (D ** -0.5)),
            "b1": _w((lambda *s: _rng.normal(s) * 0.05)(F)),
            "w2": _w((lambda *s: _rng.normal(s) * 0.05)(F, D) * (F ** -0.5)),
        }
    _B_in = _B_setup()

    return {
        "A_x": _A_in["x"],
        "A_c_kv": _A_in["c_kv"],
        "A_w_q": _A_in["w_q"],
        "A_w_uk": _A_in["w_uk"],
        "A_w_uv": _A_in["w_uv"],
        "A_w_o": _A_in["w_o"],
        "B_x": _B_in["x"],
        "B_w1": _B_in["w1"],
        "B_b1": _B_in["b1"],
        "B_w2": _B_in["w2"],
    }

def reference(A_x, A_c_kv, A_w_q, A_w_uk, A_w_uv, A_w_o, B_x, B_w1, B_b1, B_w2):
    def _A_ref(x, c_kv, w_q, w_uk, w_uv, w_o):
        B, Sq, M = x.shape[0], x.shape[1], x.shape[2]
        Sk = c_kv.shape[1]
        H, D = w_q.shape[1], w_q.shape[2]
        q = jnp.einsum("bqm,mhd->bhqd", x, w_q)
        k = jnp.einsum("bkc,chd->bhkd", c_kv, w_uk)
        v = jnp.einsum("bkc,chd->bhkd", c_kv, w_uv)
        scores = jnp.einsum("bhqd,bhkd->bhqk", q, k) * (D ** -0.5)
        off = Sk - Sq
        qi = jnp.arange(Sq)[:, None]
        kj = jnp.arange(Sk)[None, :]
        cmask = kj <= (qi + off)
        scores = jnp.where(cmask[None, None], scores, -1e9)
        p = _softmax(scores, axis=-1)
        ctx = jnp.einsum("bhqk,bhkd->bhqd", p, v)
        return jnp.einsum("bhqd,hdm->bqm", ctx, w_o)

    def _B_ref(x, w1, b1, w2):
        h = jnp.einsum("bsd,df->bsf", x, w1) + b1
        sp = jnp.log1p(jnp.exp(-jnp.abs(h))) + jnp.where(h > 0, h, jnp.zeros_like(h))
        act = h * jnp.tanh(sp)
        return jnp.einsum("bsf,fd->bsd", act, w2)

    x = A_x
    h = x + _A_ref(_layernorm(x, axis=-1), A_c_kv, A_w_q, A_w_uk, A_w_uv, A_w_o)
    h2 = h + _B_ref(_layernorm(h, axis=-1), B_w1, B_b1, B_w2)
    return h2
```

```python
import functools

import jax
import jax.numpy as jnp
from jax import lax
import jax.experimental.pallas as pl
import jax.experimental.pallas.tpu as pltpu

_BF16 = jnp.bfloat16
_F32 = jnp.float32
_NT = (((1,), (1,)), ((), ()))
_NEG = -1e30
_LANES = 128
_GROUP = 8

_KV_CHUNK = 1024
_RELAYOUT_ROWS = 16
_NUM_SEMS = 2
_MLP_TAIL = (512, 256)


def _layernorm(x, eps=1e-5):
    mean = jnp.mean(x, axis=-1, keepdims=True)
    xc = x - mean
    var = jnp.mean(xc * xc, axis=-1, keepdims=True)
    return xc / jnp.sqrt(var + eps)


def _kernel(
    x_hbm, ckv_hbm, wq_hbm, wuk_hbm, wuv_hbm, wo_hbm, w1_hbm, b1_hbm, w2_hbm,
    o_ref,
    x_v, b1_v, ckv_v, wq_v, wuk_v, wuv_v, wo_v, w1_v, w2d, q_s, acc_s, m_s, l_s,
    sems, *w2_v,
    tk, mb, w2_edges,
):
    B, Sk, Dc = ckv_hbm.shape
    M, H, D = wq_hbm.shape
    Fd = w1_hbm.shape[1]
    G = H // _GROUP
    GD = _GROUP * D
    n_chunks = Sk // tk
    n_sems = sems.shape[0]

    stream = [(wq_hbm, wq_v), (wuk_hbm, wuk_v)]
    stream += [
        (ckv_hbm.at[:, pl.ds(i * tk, tk)], ckv_v.at[i]) for i in range(n_chunks)
    ]
    stream += [(wuv_hbm, wuv_v), (wo_hbm, wo_v), (w1_hbm, w1_v)]
    stream += [
        (w2_hbm.at[pl.ds(lo, hi - lo)], dst)
        for lo, hi, dst in zip(w2_edges[:-1], w2_edges[1:], w2_v)
    ]
    copies = [
        pltpu.make_async_copy(src, dst, sems.at[n % n_sems])
        for n, (src, dst) in enumerate(stream)
    ]
    copy_x = pltpu.make_async_copy(x_hbm, x_v, sems.at[0])
    copy_b1 = pltpu.make_async_copy(b1_hbm, b1_v, sems.at[0])
    pending = iter(range(len(copies)))

    def await_next():
        n = next(pending)
        copies[n].wait()
        if n + n_sems < len(copies):
            copies[n + n_sems].start()

    copies[0].start()
    copy_x.start()
    copy_b1.start()
    for n in range(1, n_sems):
        copies[n].start()

    def to_2d(src):
        def block(i, carry):
            r0 = pl.multiple_of(i * mb, mb)
            t = jnp.swapaxes(src[pl.ds(r0, mb)], 0, 1)
            for h in range(H):
                w2d[pl.ds(r0, mb), h * D:(h + 1) * D] = t[h]
            return carry

        lax.fori_loop(0, src.shape[0] // mb, block, 0)

    def group_cols(ref, g):
        return ref[:, g * GD:(g + 1) * GD]

    row = lax.broadcasted_iota(jnp.int32, (2 * _GROUP, GD), 0)
    col = lax.broadcasted_iota(jnp.int32, (2 * _GROUP, GD), 1)
    own_head = (col // D) == (row % _GROUP)
    first_batch = lax.broadcasted_iota(jnp.int32, (2 * _GROUP, M), 0) < _GROUP

    copy_x.wait()
    copy_b1.wait()
    await_next()
    xf = x_v[...].astype(_F32)
    x16 = jnp.where(first_batch, xf[0:1], xf[1:2])
    xn16 = _layernorm(x16).astype(_BF16)
    to_2d(wq_v)
    q_rows = []
    for g in range(G):
        q16 = jnp.dot(xn16, group_cols(w2d, g), preferred_element_type=_F32)
        q_rows.append(jnp.where(own_head, q16, 0.0).astype(_BF16))

    await_next()
    to_2d(wuk_v)
    for g in range(G):
        qa = lax.dot_general(
            q_rows[g], group_cols(w2d, g), _NT, preferred_element_type=_F32
        ) * (D ** -0.5)
        for b in range(B):
            acc_s[b, g * _GROUP:(g + 1) * _GROUP, :] = qa[b * _GROUP:(b + 1) * _GROUP]
    q_s[...] = acc_s[...].astype(_BF16)
    acc_s[...] = jnp.zeros(acc_s.shape, _F32)
    m_s[...] = jnp.full(m_s.shape, _NEG, _F32)
    l_s[...] = jnp.zeros(l_s.shape, _F32)

    for i in range(n_chunks):
        await_next()
        for b in range(B):
            c = ckv_v[i, b]
            s = lax.dot_general(q_s[b], c, _NT, preferred_element_type=_F32)
            m_prev = m_s[b]
            m_new = jnp.maximum(m_prev, jnp.max(s, axis=-1, keepdims=True))
            alpha = jnp.exp(m_prev - m_new)
            p = jnp.exp(s - m_new[:, 0:1])
            l_s[b] = l_s[b] * alpha + jnp.sum(p, axis=-1, keepdims=True)
            m_s[b] = m_new
            pc = jnp.dot(p.astype(_BF16), c, preferred_element_type=_F32)
            acc_s[b] = acc_s[b] * alpha[:, 0:1] + pc

    await_next()
    to_2d(wuv_v)
    ctx_rows = []
    for g in range(G):
        heads = slice(g * _GROUP, (g + 1) * _GROUP)
        lat = jnp.concatenate(
            [acc_s[b, heads, :] / l_s[b, heads, 0:1] for b in range(B)], axis=0
        ).astype(_BF16)
        c16 = jnp.dot(lat, group_cols(w2d, g), preferred_element_type=_F32)
        ctx_rows.append(jnp.where(own_head, c16, 0.0).astype(_BF16))

    await_next()
    out16 = jnp.zeros((2 * _GROUP, M), _F32)
    for g in range(G):
        wo_g = wo_v[g * _GROUP:(g + 1) * _GROUP].reshape(GD, M)
        out16 = out16 + jnp.dot(ctx_rows[g], wo_g, preferred_element_type=_F32)
    out0 = jnp.sum(out16[0:_GROUP], axis=0, keepdims=True)
    out1 = jnp.sum(out16[_GROUP:2 * _GROUP], axis=0, keepdims=True)
    h16 = x16 + jnp.where(first_batch, out0, out1)
    hn16 = _layernorm(h16).astype(_BF16)

    await_next()
    u = jnp.dot(hn16, w1_v[...], preferred_element_type=_F32)
    b1 = b1_v[...].astype(_F32)
    u = jnp.concatenate(
        [u[:, t * _LANES:(t + 1) * _LANES] + b1[t:t + 1, :]
         for t in range(Fd // _LANES)],
        axis=1,
    )
    softplus = jnp.log1p(jnp.exp(-jnp.abs(u))) + jnp.where(u > 0, u, 0.0)
    act = (u * jnp.tanh(softplus)).astype(_BF16)

    y16 = h16
    for lo, hi, w2_piece in zip(w2_edges[:-1], w2_edges[1:], w2_v):
        await_next()
        y16 = y16 + jnp.dot(act[:, lo:hi], w2_piece[...], preferred_element_type=_F32)

    is_row0 = lax.broadcasted_iota(jnp.int32, (_GROUP, M), 0) == 0
    y8 = jnp.where(is_row0, y16[0:_GROUP], y16[_GROUP:2 * _GROUP])
    o_ref[...] = y8[0:B].astype(o_ref.dtype)


def _w2_edges(f, tail):
    edges = [f]
    for rows in reversed(tail):
        if rows < edges[0]:
            edges.insert(0, edges[0] - rows)
    return (0,) + tuple(edges)


def _run(x, c_kv, w_q, w_uk, w_uv, w_o, w1, b1, w2, *, tk, mb, n_sems, mlp_tail):
    B, Sq, M = x.shape
    _, Sk, Dc = c_kv.shape
    _, H, D = w_q.shape
    Fd = w1.shape[1]
    assert B == 2 and Sq == 1, "one decode step for two sequences"
    assert D == _LANES and H % _GROUP == 0 and Dc == M
    assert Sk % tk == 0 and Fd % _LANES == 0 and M % mb == 0
    w2_edges = _w2_edges(Fd, mlp_tail)

    hbm = pl.BlockSpec(memory_space=pl.ANY)
    scratch = [
        pltpu.VMEM((B, M), _BF16),
        pltpu.VMEM((Fd // _LANES, _LANES), _BF16),
        pltpu.VMEM((Sk // tk, B, tk, Dc), _BF16),
        pltpu.VMEM((M, H, D), _BF16),
        pltpu.VMEM((Dc, H, D), _BF16),
        pltpu.VMEM((Dc, H, D), _BF16),
        pltpu.VMEM((H, D, M), _BF16),
        pltpu.VMEM((M, Fd), _BF16),
        pltpu.VMEM((Dc, H * D), _BF16),
        pltpu.VMEM((B, H, Dc), _BF16),
        pltpu.VMEM((B, H, Dc), _F32),
        pltpu.VMEM((B, H, _LANES), _F32),
        pltpu.VMEM((B, H, _LANES), _F32),
        pltpu.SemaphoreType.DMA((n_sems,)),
    ]
    scratch += [
        pltpu.VMEM((hi - lo, M), _BF16)
        for lo, hi in zip(w2_edges[:-1], w2_edges[1:])
    ]
    out = pl.pallas_call(
        functools.partial(_kernel, tk=tk, mb=mb, w2_edges=w2_edges),
        out_shape=jax.ShapeDtypeStruct((B, M), x.dtype),
        in_specs=[hbm] * 9,
        out_specs=pl.BlockSpec(memory_space=pltpu.VMEM),
        scratch_shapes=scratch,
        compiler_params=pltpu.CompilerParams(vmem_limit_bytes=64 * 1024 * 1024),
    )(
        x.reshape(B, M), c_kv, w_q, w_uk, w_uv, w_o,
        w1, b1.reshape(Fd // _LANES, _LANES), w2,
    )
    return out.reshape(B, Sq, M)


@jax.jit
def pallas_sequential_preLN__compressed_kv_cla__dense_activation_mish__decode_kernel(
    A_x: jax.Array,
    A_c_kv: jax.Array,
    A_w_q: jax.Array,
    A_w_uk: jax.Array,
    A_w_uv: jax.Array,
    A_w_o: jax.Array,
    B_x: jax.Array,
    B_w1: jax.Array,
    B_b1: jax.Array,
    B_w2: jax.Array,
):
    del B_x
    return _run(
        A_x, A_c_kv, A_w_q, A_w_uk, A_w_uv, A_w_o, B_w1, B_b1, B_w2,
        tk=_KV_CHUNK, mb=_RELAYOUT_ROWS, n_sems=_NUM_SEMS, mlp_tail=_MLP_TAIL,
    )
```

```python
import functools

import jax
import jax.numpy as jnp
from jax import lax
import jax.experimental.pallas as pl
import jax.experimental.pallas.tpu as pltpu

_BF16 = jnp.bfloat16
_F32 = jnp.float32
_NT = (((1,), (1,)), ((), ()))
_NEG = -3.4028234663852886e38
_LANES = 128
_GROUP = 8

_KV_CHUNK = 1024
_RELAYOUT_ROWS = 16
_NUM_SEMS = 2
_MLP_TAIL = (384, 128)


def _layernorm(x, eps=1e-5):
    mean = jnp.mean(x, axis=-1, keepdims=True)
    xc = x - mean
    var = jnp.mean(xc * xc, axis=-1, keepdims=True)
    return xc / jnp.sqrt(var + eps)


def _kernel(
    x_hbm, ckv_hbm, wq_hbm, wuk_hbm, wuv_hbm, wo_hbm, w1_hbm, b1_hbm, w2_hbm,
    o_ref,
    x_v, b1_v, ckv_v, wq_v, wuk_v, wuv_v, wo_v, w1_v, w2d, q_s, acc_s, m_s, l_s,
    sems, *w2_v,
    tk, mb, w2_edges,
):
    B, Sk, Dc = ckv_hbm.shape
    M, H, D = wq_hbm.shape
    Fd = w1_hbm.shape[1]
    G = H // _GROUP
    GD = _GROUP * D
    n_chunks = Sk // tk
    n_sems = sems.shape[0]

    stream = [(wq_hbm, wq_v), (wuk_hbm, wuk_v)]
    stream += [
        (ckv_hbm.at[:, pl.ds(i * tk, tk)], ckv_v.at[i]) for i in range(n_chunks)
    ]
    stream += [(wuv_hbm, wuv_v), (wo_hbm, wo_v), (w1_hbm, w1_v)]
    stream += [
        (w2_hbm.at[pl.ds(lo, hi - lo)], dst)
        for lo, hi, dst in zip(w2_edges[:-1], w2_edges[1:], w2_v)
    ]
    copies = [
        pltpu.make_async_copy(src, dst, sems.at[n % n_sems])
        for n, (src, dst) in enumerate(stream)
    ]
    copy_x = pltpu.make_async_copy(x_hbm, x_v, sems.at[0])
    copy_b1 = pltpu.make_async_copy(b1_hbm, b1_v, sems.at[0])
    pending = iter(range(len(copies)))

    def await_next():
        n = next(pending)
        copies[n].wait()
        if n + n_sems < len(copies):
            copies[n + n_sems].start()

    copies[0].start()
    copy_x.start()
    copy_b1.start()
    for n in range(1, n_sems):
        copies[n].start()

    def to_2d(src):
        def block(i, carry):
            r0 = pl.multiple_of(i * mb, mb)
            t = jnp.swapaxes(src[pl.ds(r0, mb)], 0, 1)
            for h in range(H):
                w2d[pl.ds(r0, mb), h * D:(h + 1) * D] = t[h]
            return carry

        lax.fori_loop(0, src.shape[0] // mb, block, 0)

    def group_cols(ref, g):
        return ref[:, g * GD:(g + 1) * GD]

    row = lax.broadcasted_iota(jnp.int32, (2 * _GROUP, GD), 0)
    col = lax.broadcasted_iota(jnp.int32, (2 * _GROUP, GD), 1)
    own_head = (col // D) == (row % _GROUP)
    first_batch = lax.broadcasted_iota(jnp.int32, (2 * _GROUP, M), 0) < _GROUP

    copy_x.wait()
    copy_b1.wait()
    await_next()
    xf = x_v[...].astype(_F32)
    x16 = jnp.where(first_batch, xf[0:1], xf[1:2])
    xn16 = _layernorm(x16).astype(_BF16)
    to_2d(wq_v)
    q_rows = []
    for g in range(G):
        q16 = jnp.dot(xn16, group_cols(w2d, g), preferred_element_type=_F32)
        q_rows.append(jnp.where(own_head, q16, 0.0).astype(_BF16))

    await_next()
    to_2d(wuk_v)
    for g in range(G):
        qa = lax.dot_general(
            q_rows[g], group_cols(w2d, g), _NT, preferred_element_type=_F32
        ) * (D ** -0.5)
        for b in range(B):
            acc_s[b, g * _GROUP:(g + 1) * _GROUP, :] = qa[b * _GROUP:(b + 1) * _GROUP]
    q_s[...] = acc_s[...].astype(_BF16)
    acc_s[...] = jnp.zeros(acc_s.shape, _F32)
    m_s[...] = jnp.full(m_s.shape, _NEG, _F32)
    l_s[...] = jnp.zeros(l_s.shape, _F32)

    for i in range(n_chunks):
        await_next()
        for b in range(B):
            c = ckv_v[i, b]
            s = lax.dot_general(q_s[b], c, _NT, preferred_element_type=_F32)
            m_prev = m_s[b]
            m_new = jnp.maximum(m_prev, jnp.max(s, axis=-1, keepdims=True))
            alpha = jnp.exp(m_prev - m_new)
            p = jnp.exp(s - m_new[:, 0:1])
            l_s[b] = l_s[b] * alpha + jnp.sum(p, axis=-1, keepdims=True)
            m_s[b] = m_new
            pc = jnp.dot(p.astype(_BF16), c, preferred_element_type=_F32)
            acc_s[b] = acc_s[b] * alpha[:, 0:1] + pc

    await_next()
    to_2d(wuv_v)
    ctx_rows = []
    for g in range(G):
        heads = slice(g * _GROUP, (g + 1) * _GROUP)
        lat = jnp.concatenate(
            [acc_s[b, heads, :] / l_s[b, heads, 0:1] for b in range(B)], axis=0
        ).astype(_BF16)
        c16 = jnp.dot(lat, group_cols(w2d, g), preferred_element_type=_F32)
        ctx_rows.append(jnp.where(own_head, c16, 0.0).astype(_BF16))

    await_next()
    out16 = jnp.zeros((2 * _GROUP, M), _F32)
    for g in range(G):
        wo_g = wo_v[g * _GROUP:(g + 1) * _GROUP].reshape(GD, M)
        out16 = out16 + jnp.dot(ctx_rows[g], wo_g, preferred_element_type=_F32)
    out0 = jnp.sum(out16[0:_GROUP], axis=0, keepdims=True)
    out1 = jnp.sum(out16[_GROUP:2 * _GROUP], axis=0, keepdims=True)
    h16 = x16 + jnp.where(first_batch, out0, out1)
    hn16 = _layernorm(h16).astype(_BF16)

    await_next()
    u = jnp.dot(hn16, w1_v[...], preferred_element_type=_F32)
    b1 = b1_v[...].astype(_F32)
    u = jnp.concatenate(
        [u[:, t * _LANES:(t + 1) * _LANES] + b1[t:t + 1, :]
         for t in range(Fd // _LANES)],
        axis=1,
    )
    softplus = jnp.log1p(jnp.exp(-jnp.abs(u))) + jnp.where(u > 0, u, 0.0)
    act = (u * jnp.tanh(softplus)).astype(_BF16)

    y16 = h16
    for lo, hi, w2_piece in zip(w2_edges[:-1], w2_edges[1:], w2_v):
        await_next()
        y16 = y16 + jnp.dot(act[:, lo:hi], w2_piece[...], preferred_element_type=_F32)

    is_row0 = lax.broadcasted_iota(jnp.int32, (_GROUP, M), 0) == 0
    y8 = jnp.where(is_row0, y16[0:_GROUP], y16[_GROUP:2 * _GROUP])
    o_ref[...] = y8[0:B].astype(o_ref.dtype)


def _w2_edges(f, tail):
    edges = [f]
    for rows in reversed(tail):
        if rows < edges[0]:
            edges.insert(0, edges[0] - rows)
    return (0,) + tuple(edges)


def _run(x, c_kv, w_q, w_uk, w_uv, w_o, w1, b1, w2, *, tk, mb, n_sems, mlp_tail):
    B, Sq, M = x.shape
    _, Sk, Dc = c_kv.shape
    _, H, D = w_q.shape
    Fd = w1.shape[1]
    assert B == 2 and Sq == 1, "one decode step for two sequences"
    assert D == _LANES and H % _GROUP == 0 and Dc == M
    assert Sk % tk == 0 and Fd % _LANES == 0 and M % mb == 0
    assert all(
        a.dtype == _BF16 for a in (x, c_kv, w_q, w_uk, w_uv, w_o, w1, b1, w2)
    ), "operands are staged in VMEM as bfloat16"
    w2_edges = _w2_edges(Fd, mlp_tail)

    hbm = pl.BlockSpec(memory_space=pl.ANY)
    scratch = [
        pltpu.VMEM((B, M), _BF16),
        pltpu.VMEM((Fd // _LANES, _LANES), _BF16),
        pltpu.VMEM((Sk // tk, B, tk, Dc), _BF16),
        pltpu.VMEM((M, H, D), _BF16),
        pltpu.VMEM((Dc, H, D), _BF16),
        pltpu.VMEM((Dc, H, D), _BF16),
        pltpu.VMEM((H, D, M), _BF16),
        pltpu.VMEM((M, Fd), _BF16),
        pltpu.VMEM((Dc, H * D), _BF16),
        pltpu.VMEM((B, H, Dc), _BF16),
        pltpu.VMEM((B, H, Dc), _F32),
        pltpu.VMEM((B, H, _LANES), _F32),
        pltpu.VMEM((B, H, _LANES), _F32),
        pltpu.SemaphoreType.DMA((n_sems,)),
    ]
    scratch += [
        pltpu.VMEM((hi - lo, M), _BF16)
        for lo, hi in zip(w2_edges[:-1], w2_edges[1:])
    ]
    out = pl.pallas_call(
        functools.partial(_kernel, tk=tk, mb=mb, w2_edges=w2_edges),
        out_shape=jax.ShapeDtypeStruct((B, M), x.dtype),
        in_specs=[hbm] * 9,
        out_specs=pl.BlockSpec(memory_space=pltpu.VMEM),
        scratch_shapes=scratch,
        compiler_params=pltpu.CompilerParams(vmem_limit_bytes=64 * 1024 * 1024),
    )(
        x.reshape(B, M), c_kv, w_q, w_uk, w_uv, w_o,
        w1, b1.reshape(Fd // _LANES, _LANES), w2,
    )
    return out.reshape(B, Sq, M)


@jax.jit
def pallas_sequential_preLN__compressed_kv_cla__dense_activation_mish__decode_kernel(
    A_x: jax.Array,
    A_c_kv: jax.Array,
    A_w_q: jax.Array,
    A_w_uk: jax.Array,
    A_w_uv: jax.Array,
    A_w_o: jax.Array,
    B_x: jax.Array,
    B_w1: jax.Array,
    B_b1: jax.Array,
    B_w2: jax.Array,
):
    del B_x
    return _run(
        A_x, A_c_kv, A_w_q, A_w_uk, A_w_uv, A_w_o, B_w1, B_b1, B_w2,
        tk=_KV_CHUNK, mb=_RELAYOUT_ROWS, n_sems=_NUM_SEMS, mlp_tail=_MLP_TAIL,
    )
```
